```python
import os as _os
_os.environ.setdefault("JAX_PLATFORMS", "cpu")
import jax
import jax.numpy as jnp

def _softmax(x, axis=-1):
    return jax.nn.softmax(x, axis=axis)
def _gelu(x):
    return jax.nn.gelu(x, approximate=True)
def _silu(x):
    return jax.nn.silu(x)
def _sigmoid(x):
    return jax.nn.sigmoid(x)
def _layernorm(x, axis=-1, eps=1e-5):
    m = jnp.mean(x, axis=axis, keepdims=True)
    v = jnp.var(x, axis=axis, keepdims=True)
    return (x - m) / jnp.sqrt(v + eps)
def _scatter_add(tgt, idx, src, axis=0):
    return tgt.at[idx].add(src)
def _segment_sum(src, seg, n):
    return jax.ops.segment_sum(src, seg, n)
class _Rng:
    def __init__(self, key):
        self._k = key
    def _next(self):
        self._k, sub = jax.random.split(self._k)
        return sub
    def normal(self, shape):
        return jax.random.normal(self._next(), shape, dtype=jnp.bfloat16)
    def randint(self, lo, hi, shape):
        return jax.random.randint(self._next(), shape, lo, hi, dtype=jnp.int32)
    def uniform(self, shape, lo=0.0, hi=1.0):
        return jax.random.uniform(self._next(), shape, jnp.bfloat16, lo, hi)
    def permutation(self, n):
        return jax.random.permutation(self._next(), n)


kernel_name = 'gated_mix__grouped_kv_mqa__swiglu_ffn__prompt'

def setup_inputs():
    _rng = _Rng(jax.random.key(int.from_bytes(__import__("os").urandom(4), "little")))
    _w = (lambda a: (lambda t: t.astype(jnp.bfloat16) if jnp.issubdtype(t.dtype, jnp.floating) else t)(jnp.asarray(a)))
    def _A_setup():
        B, S, D, H = 1, 2048, 512, 32
        Dh = D // H
        return {
            "x": _w((lambda *s: _rng.normal(s) * 0.05)(B, S, D)),
            "wq": _w((lambda *s: _rng.normal(s) * 0.4)(D, H * Dh)),
            "wk": _w((lambda *s: _rng.normal(s) * 0.4)(D, Dh)),
            "wv": _w((lambda *s: _rng.normal(s) * 0.05)(D, Dh)),
            "wo": _w((lambda *s: _rng.normal(s) * 0.05)(H * Dh, D)),
        }
    _A_in = _A_setup()

    def _B_setup():
        B, S, D, F = 1, 2048, 512, 1792
        return {
            "x": _w((lambda *s: _rng.normal(s) * 0.05)(B, S, D)),
            "w_gate": _w((lambda *s: _rng.normal(s) * 0.05)(D, F)),
            "w_up": _w((lambda *s: _rng.normal(s) * 0.05)(D, F)),
            "w_down": _w((lambda *s: _rng.normal(s) * 0.05)(F, D)),
        }
    _B_in = _B_setup()

    return {
        "A_x": _A_in["x"],
        "A_wq": _A_in["wq"],
        "A_wk": _A_in["wk"],
        "A_wv": _A_in["wv"],
        "A_wo": _A_in["wo"],
        "B_x": _B_in["x"],
        "B_w_gate": _B_in["w_gate"],
        "B_w_up": _B_in["w_up"],
        "B_w_down": _B_in["w_down"],
        "gate_w": _w((lambda *s: _rng.normal(s) * 0.05)(512) * 16.0),
    }

def reference(A_x, A_wq, A_wk, A_wv, A_wo, B_x, B_w_gate, B_w_up, B_w_down, gate_w):
    def _A_ref(x, wq, wk, wv, wo):
        B, S, D = x.shape
        H = 32
        Dh = D // H
        q = (lambda x, *d: x.transpose(*d))((x @ wq).reshape(B, S, H, Dh), 0, 2, 1, 3)
        k = x @ wk
        v = x @ wv
        scores = jnp.einsum("bhqd,bkd->bhqk", q, k) * (Dh ** -0.5)
        p = _softmax(scores, axis=-1)
        o = jnp.einsum("bhqk,bkd->bhqd", p, v)
        return (lambda x, *d: x.transpose(*d))(o, 0, 2, 1, 3).reshape(B, S, H * Dh) @ wo

    def _B_ref(x, w_gate, w_up, w_down):
        g = _silu(x @ w_gate)
        u = x @ w_up
        return (g * u) @ w_down

    x = A_x
    g = _sigmoid((x * gate_w).sum(-1, keepdims=True))
    a = _A_ref(x, A_wq, A_wk, A_wv, A_wo)
    b = _B_ref(x, B_w_gate, B_w_up, B_w_down)
    return g * a + (1 - g) * b
```

```python
import functools, math
import jax
import jax.numpy as jnp
from jax import lax
import jax.experimental.pallas as pl
import jax.experimental.pallas.tpu as pltpu

H = 32
DH = 16
LOG2E = 1.4426950408889634
f32 = jnp.float32
bf16 = jnp.bfloat16
u32 = jnp.uint32
CK = 128
NT = (((1,), (1,)), ((), ()))
TN = (((0,), (0,)), ((), ()))


def make_kernel(S, D, F, TQ, FC, G, order, nb_per_dot, wo_pos, qmode, xw):
    NQ = S // TQ
    NC = S // CK
    NF = F // FC
    scale = (DH ** -0.5) * LOG2E

    def kernel(x_hbm, wq_hbm, wkT_hbm, wvT_hbm, wo_hbm, wg_hbm, wu_hbm, wd_hbm, gw_ref,
               o_ref, x_sc, wq_sc, wkv_sc, wo_sc, wg_sc, wu_sc, wd_sc,
               k_sc, vT_sc, qT_sc, oT_sc, sems, *sm):
        s_scs = sm[:G]
        m_scs = sm[G:]
        i = pl.program_id(0)

        def x_copy(t):
            return pltpu.make_async_copy(x_hbm.at[pl.ds(t * TQ, TQ), :], x_sc.at[pl.ds(t * TQ, TQ), :], sems.at[t])
        wq_copy = pltpu.make_async_copy(wq_hbm, wq_sc, sems.at[NQ])
        wk_copy = pltpu.make_async_copy(wkT_hbm, wkv_sc.at[pl.ds(0, DH), :], sems.at[NQ + 1])
        wv_copy = pltpu.make_async_copy(wvT_hbm, wkv_sc.at[pl.ds(DH, DH), :], sems.at[NQ + 2])
        late_copies = [
            pltpu.make_async_copy(wg_hbm, wg_sc, sems.at[NQ + 3]),
            pltpu.make_async_copy(wu_hbm, wu_sc, sems.at[NQ + 4]),
            pltpu.make_async_copy(wd_hbm, wd_sc, sems.at[NQ + 5]),
            pltpu.make_async_copy(wo_hbm, wo_sc, sems.at[NQ + 6]),
        ]

        def a_chunk(head, col0, g, c):
            qT = pltpu.bitcast(qT_sc[pl.ds(pl.multiple_of(head * 8, 8), 8), pl.ds(col0, TQ)], bf16)
            kk = pltpu.bitcast(k_sc[c * CK // 2:(c + 1) * CK // 2, :], bf16)
            s = jnp.dot(kk, qT, preferred_element_type=f32)
            s_scs[g][c * CK:(c + 1) * CK, :] = s
            return s

        def max_acc(mn, s):
            for j in range(CK // 8):
                v = s[8 * j:8 * j + 8, :]
                mn = v if mn is None else jnp.maximum(mn, v)
            return mn

        def b_chunk(s, m, c, l):
            ps = [jnp.exp2(s[8 * j:8 * j + 8, :] - m) for j in range(16)]
            for v in ps:
                l = v if l is None else l + v
            pb = jnp.concatenate([ps[2 * j + e] for j in reversed(range(8)) for e in range(2)], axis=0).astype(bf16)
            vT = pltpu.bitcast(vT_sc[:, c * CK:(c + 1) * CK], bf16)
            o = jnp.dot(vT, pb, preferred_element_type=f32)
            return l, o

        class St:
            pass

        def start(g, a_head, a_col, b_head):
            st = St()
            st.g = g; st.a_head = a_head; st.a_col = a_col; st.b_head = b_head
            st.m = None
            st.mn = None; st.l = None; st.o = None
            return st

        def step(st, c):
            if st.b_head is not None:
                if st.m is None:
                    st.m = m_scs[st.g][...]
                sb = s_scs[st.g][c * CK:(c + 1) * CK, :]
            if st.a_head is not None:
                sa = a_chunk(st.a_head, st.a_col, st.g, c)
                st.mn = max_acc(st.mn, sa)
            if st.b_head is not None:
                st.l, oc = b_chunk(sb, st.m, c, st.l)
                st.o = oc if st.o is None else st.o + oc

        def finish(st):
            if st.a_head is not None:
                m_scs[st.g][...] = jnp.broadcast_to(jnp.max(st.mn, axis=0, keepdims=True), (8, TQ))
            if st.b_head is not None:
                ls = jnp.sum(st.l, axis=0, keepdims=True)
                row = st.b_head * DH
                if not isinstance(row, int):
                    row = pl.multiple_of(row, DH)
                oT_sc[pl.ds(row, DH), :] = (st.o * (1.0 / ls)).astype(oT_sc.dtype)

        def run(sts):
            if order == "seq":
                for st in sts:
                    for c in range(NC):
                        step(st, c)
                    finish(st)
            else:
                for c in range(NC):
                    for st in sts:
                        step(st, c)
                for st in sts:
                    finish(st)

        col = pl.multiple_of(i * TQ, TQ)

        @pl.when(i == 0)
        def _():
            wq_copy.start(); wk_copy.start(); wv_copy.start()
            for t in range(NQ):
                x_copy(t).start()
            wq_copy.wait(); wk_copy.wait(); wv_copy.wait()
            if qmode == "wT":
                wqT = wq_sc[...].T
            for t in range(NQ):
                if t in xw:
                    nxt = [u for u in xw if u > t]
                    for u in range(t, nxt[0] if nxt else NQ):
                        x_copy(u).wait()
                    if not nxt:
                        for cp in late_copies:
                            cp.start()
                xt = x_sc[t * TQ:(t + 1) * TQ, :]
                kvT = lax.dot_general(wkv_sc[...], xt, NT, preferred_element_type=f32)
                k = (kvT[0:DH, :] * scale).T
                kperm = jnp.concatenate([k[c * CK + 16 * j:c * CK + 16 * j + 16, :]
                                         for c in range(TQ // CK) for j in reversed(range(8))], axis=0)
                k_sc[t * TQ // 2:(t + 1) * TQ // 2, :] = pltpu.bitcast(kperm.astype(bf16), u32)
                vT_sc[:, t * TQ:(t + 1) * TQ] = pltpu.bitcast(kvT[DH:2 * DH, :].astype(bf16), u32)
                if qmode == "wT":
                    qT = lax.dot_general(wqT, xt, NT, preferred_element_type=f32)
                else:
                    qT = jnp.dot(xt, wq_sc[...], preferred_element_type=f32).T
                qT_sc[:, t * TQ:(t + 1) * TQ] = pltpu.bitcast(qT.astype(bf16), u32)

        run([start(g, g, col, None) for g in range(G)])

        def body(j, carry):
            run([start(g, (j + 1) * G + g, col, j * G + g) for g in range(G)])
            return carry
        lax.fori_loop(0, H // G - 1, body, 0)

        @pl.when(i == 0)
        def _():
            for cp in late_copies:
                cp.wait()

        sts = [start(g, None, None, H - G + g) for g in range(G)]
        pending = [(st, c) for st in sts for c in range(NC)] if order == "seq" else \
                  [(st, c) for c in range(NC) for st in sts]
        done = [0] * G
        credit = [0.0]

        def emit_b(n):
            credit[0] += n
            while credit[0] >= 1 and pending:
                credit[0] -= 1
                st, c = pending.pop(0)
                step(st, c)
                done[st.g] += 1
                if done[st.g] == NC:
                    finish(st)

        xt = x_sc[pl.ds(col, TQ), :]
        b = None
        a = None
        for f in range(NF):
            if f == wo_pos:
                emit_b(len(pending))
                a = lax.dot_general(oT_sc[...], wo_sc[...], TN, preferred_element_type=f32)
            g_ = jnp.dot(xt, wg_sc[:, f * FC:(f + 1) * FC], preferred_element_type=f32)
            emit_b(nb_per_dot)
            u = jnp.dot(xt, wu_sc[:, f * FC:(f + 1) * FC], preferred_element_type=f32)
            emit_b(nb_per_dot)
            hm = (g_ * jax.nn.sigmoid(g_) * u).astype(bf16)
            bc = jnp.dot(hm, wd_sc[f * FC:(f + 1) * FC, :], preferred_element_type=f32)
            emit_b(nb_per_dot)
            b = bc if b is None else b + bc
        assert a is not None
        gw = gw_ref[...].reshape(1, D).astype(f32)
        z = jnp.sum(xt.astype(f32) * gw, axis=-1, keepdims=True)
        gate = jax.nn.sigmoid(z)
        o_ref[...] = (gate * a + (1.0 - gate) * b).astype(o_ref.dtype)

    return kernel, NQ


_CFG = dict(TQ=512, FC=128, G=2, order="il", nb_per_dot=1, wo_pos=12, qmode="q", xw=(0, 1))


@jax.jit
def pallas_gated_mix__grouped_kv_mqa__swiglu_ffn__prompt_kernel(
    A_x, A_wq, A_wk, A_wv, A_wo, B_x, B_w_gate, B_w_up, B_w_down, gate_w):
    TQ, FC, G = _CFG["TQ"], _CFG["FC"], _CFG["G"]
    order, nb_per_dot, wo_pos = _CFG["order"], _CFG["nb_per_dot"], _CFG["wo_pos"]
    qmode, xw = _CFG["qmode"], _CFG["xw"]
    B, S, D = A_x.shape
    F = B_w_gate.shape[1]
    x = A_x.reshape(S, D)
    kernel, NQ = make_kernel(S, D, F, TQ, FC, G, order, nb_per_dot, wo_pos, qmode, list(xw))
    hbm = pl.BlockSpec(memory_space=pl.ANY)
    out = pl.pallas_call(
        kernel,
        grid=(NQ,),
        in_specs=[hbm] * 8 + [pl.BlockSpec((D,), lambda i: (0,))],
        out_specs=pl.BlockSpec((TQ, D), lambda i: (i, 0)),
        out_shape=jax.ShapeDtypeStruct((S, D), A_x.dtype),
        scratch_shapes=[
            pltpu.VMEM((S, D), bf16),
            pltpu.VMEM((D, D), bf16),
            pltpu.VMEM((2 * DH, D), bf16),
            pltpu.VMEM((D, D), bf16),
            pltpu.VMEM((D, F), bf16),
            pltpu.VMEM((D, F), bf16),
            pltpu.VMEM((F, D), bf16),
            pltpu.VMEM((S // 2, DH), u32),
            pltpu.VMEM((DH // 2, S), u32),
            pltpu.VMEM((D // 2, S), u32),
            pltpu.VMEM((D, TQ), bf16),
            pltpu.SemaphoreType.DMA((NQ + 7,)),
        ] + [pltpu.VMEM((S, TQ), f32)] * G + [pltpu.VMEM((8, TQ), f32)] * G,
        compiler_params=pltpu.CompilerParams(
            dimension_semantics=("arbitrary",),
            vmem_limit_bytes=100 * 1024 * 1024),
    )(x, A_wq, A_wk.T, A_wv.T, A_wo, B_w_gate, B_w_up, B_w_down, gate_w)
    return out.reshape(B, S, D)
```

```python
import jax
import jax.numpy as jnp
from jax import lax
import jax.experimental.pallas as pl
import jax.experimental.pallas.tpu as pltpu

H = 32
DH = 16
LOG2E = 1.4426950408889634
f32 = jnp.float32
bf16 = jnp.bfloat16
u32 = jnp.uint32
CK = 128
NT = (((1,), (1,)), ((), ()))
TN = (((0,), (0,)), ((), ()))
S_BOUND = 40.0
V_BOUND = 2.0 ** 60


def _make_kernel(S, D, F, TQ, FC, G, NB, WO_POS, NVG, NVGA, P0, P1, E, TIE, NPV, GRP):
    NQ = S // TQ
    NC = S // CK
    NF = F // FC
    NCOL = TQ // 128
    NIT = H // G - 1
    FPAR = NIT % 2
    NKB = E + max(NVG, NVGA)
    NRW = (2 * DH + D) // 16
    scale = (DH ** -0.5) * LOG2E

    def make_plan(nvg):
        first = E + nvg
        npos = (S - 16 * first) // 8
        nb = nvg * NCOL
        scheds = []
        for g in range(G):
            sched = {}
            p0 = P0 if g == 0 else 0
            p1 = P1 if g == G - 1 else 2
            for n in range(nb):
                pos = max(p0 + ((2 * n + 1) * (npos - p0 - p1)) // (2 * nb), -1)
                gi = E + (n // NCOL + (n % NCOL) * nvg // NCOL) % nvg
                sched.setdefault((pos, n % NCOL), []).append(gi)
            scheds.append(sched)
        ngr = S // 16 - first
        bounds = [16 * first + 16 * ((c * ngr) // NC) for c in range(NC + 1)]
        return first, scheds, bounds

    plan_loop = make_plan(NVG)
    plan_first = make_plan(NVGA)

    def kernel(x_hbm, wq_hbm, wkT_hbm, wvT_hbm, wo_hbm, wg_hbm, wu_hbm, wd_hbm, gw_hbm,
               o_ref, gw_sc, x_sc, wq_sc, wT_sc, wo_sc, wg_sc, wu_sc, wd_sc,
               k_sc, vT_sc, qT_sc, oT_sc, kb_sc, s_sc, qn_sc, qnext_sc, qzero_sc, pe_sc, le_sc,
               flag_sc, kn_sc, sems, *bufs):
        p_all, l_all = bufs[0:2], bufs[2:4]
        p_scs = [[pa.at[g] for g in range(G)] for pa in p_all]
        l_scs = [[la.at[g] for g in range(G)] for la in l_all]
        q_scs = [bufs[4:4 + G], bufs[4 + G:4 + 2 * G]]
        qb_scs = [bufs[4 + 2 * G:4 + 3 * G], bufs[4 + 3 * G:]]
        i = pl.program_id(0)
        col = pl.multiple_of(i * TQ, TQ)
        inext = jnp.minimum(i + 1, NQ - 1)
        coln = pl.multiple_of(inext * TQ, TQ)
        coln2 = pl.multiple_of(jnp.minimum(i + 2, NQ - 1) * TQ, TQ)

        def x_copy(t):
            rows = pl.ds(t * TQ, TQ)
            return pltpu.make_async_copy(x_hbm.at[rows, :], x_sc.at[rows, :], sems.at[t])

        wq_copy = pltpu.make_async_copy(wq_hbm, wq_sc, sems.at[NQ])
        wk_copy = pltpu.make_async_copy(wkT_hbm, wT_sc.at[pl.ds(0, DH), :], sems.at[NQ + 1])
        wv_copy = pltpu.make_async_copy(wvT_hbm, wT_sc.at[pl.ds(DH, DH), :], sems.at[NQ + 2])
        late_copies = [
            pltpu.make_async_copy(wg_hbm, wg_sc, sems.at[NQ + 3]),
            pltpu.make_async_copy(wu_hbm, wu_sc, sems.at[NQ + 4]),
            pltpu.make_async_copy(wd_hbm, wd_sc, sems.at[NQ + 5]),
            pltpu.make_async_copy(wo_hbm, wo_sc, sems.at[NQ + 6]),
            pltpu.make_async_copy(gw_hbm, gw_sc, sems.at[NQ + 7]),
        ]

        def aligned(v, m):
            return v if isinstance(v, int) else pl.multiple_of(v, m)

        def lanes(t):
            return slice(t * 128, (t + 1) * 128)

        def pack(v):
            return pltpu.bitcast(v.astype(bf16), u32)

        def load_qT(head, c0):
            return pltpu.bitcast(qT_sc[pl.ds(aligned(head * 8, 8), 8), pl.ds(c0, TQ)], bf16)

        def stage_q(par, g, head, c0):
            qv = load_qT(head, c0)
            q_scs[par][g][...] = qv.astype(f32)
            qb_scs[par][g][...] = pltpu.bitcast(qv, u32)

        def q_rows(cache, q_ref, row0, t):
            if (row0, t) not in cache:
                cache[(row0, t)] = jnp.stack(
                    [jnp.broadcast_to(q_ref[row0 + d:row0 + d + 1, lanes(t)], (8, 128)) for d in range(DH)]
                )[:, None]
            return cache[(row0, t)]

        def chain_sum(acc, v):
            if acc is not None:
                v = jnp.concatenate([acc[None], v], axis=0)
            return jnp.sum(v, axis=0)

        def vpu_scores(qb, gi):
            kb = kb_sc[:, 2 * gi:2 * gi + 2]
            acc = chain_sum(None, kb[0:DH // 2] * qb[0:DH // 2])
            acc = chain_sum(acc, kb[DH // 2:] * qb[DH // 2:])
            return acc.reshape(16, 128)

        def anchored(col_u32, outs, never):
            rows = []
            prev = 0
            for r in sorted(outs):
                if r > prev:
                    rows.append(col_u32[8 * prev:8 * r, :])
                piece = col_u32[8 * r:8 * r + 8, :]
                rows.append(jnp.where(never, pltpu.bitcast(outs[r], piece.dtype), piece))
                prev = r + 1
            if 8 * prev < col_u32.shape[0]:
                rows.append(col_u32[8 * prev:, :])
            return jnp.concatenate(rows, axis=0)

        def anchored_lhs(lhs_u32, outs, never):
            if outs:
                lhs_u32 = jnp.concatenate(
                    [anchored(lhs_u32[:, 0:128], outs, never), lhs_u32[:, 128:]], axis=1)
            return pltpu.bitcast(lhs_u32, bf16)

        def a_chunk(head, q_ref, qb_ref, p_ref, c, l, plan, g, cache):
            first, scheds, bounds = plan
            lo, hi = bounds[c], bounds[c + 1]
            qT = pltpu.bitcast(qb_ref[...], bf16)
            kk = pltpu.bitcast(k_sc[lo // 2:hi // 2, :], bf16)
            p = jnp.exp2(jnp.dot(kk, qT, preferred_element_type=f32))
            pcols = [p[:, lanes(t)] for t in range(NCOL)]
            for t in range(NCOL):
                p_ref[lo // 2:hi // 2, lanes(t)] = pack(pcols[t])
            l = list(l)
            base = (lo - 16 * first) // 8
            nv = (hi - lo) // 8

            def bursts(pos, t):
                for gi in scheds[g].get((pos, t), []):
                    v = jnp.exp2(vpu_scores(q_rows(cache, q_ref, 0, t), gi))
                    p_ref[gi * 8:gi * 8 + 8, lanes(t)] = pack(v)
                    l[t] = chain_sum(l[t], v.reshape(2, 8, 128))

            if base == 0:
                for t in range(NCOL):
                    bursts(-1, t)
            done = [0] * NCOL
            p3 = [pc.reshape(nv, 8, 128) for pc in pcols]
            for j in range(nv):
                for t in range(NCOL):
                    if (base + j, t) in scheds[g] or j == nv - 1:
                        l[t] = chain_sum(l[t], p3[t][done[t]:j + 1])
                        done[t] = j + 1
                        bursts(base + j, t)
            if c == 1:
                p_ref[0:8 * E, :] = pe_sc[head]
                le = le_sc[head]
                for t in range(NCOL):
                    l[t] = l[t] + le[:, lanes(t)]
            return l

        def store_o(head, o, l):
            r = jnp.broadcast_to(1.0 / jnp.sum(l, axis=0, keepdims=True), (8, TQ))
            on = jnp.concatenate([o[0:8, :] * r, o[8:16, :] * r], axis=0)
            oT_sc[pl.ds(aligned(head * DH, DH), DH), :] = on.astype(bf16)

        def stream(g, rd, a_head, b_head):
            return dict(g=g, rd=rd, a=a_head, b=b_head, l=[None] * NCOL, o=None, q={})

        def step_a(st, c):
            g, rd = st["g"], st["rd"]
            st["l"] = a_chunk(st["a"], q_scs[rd][g], qb_scs[rd][g], p_scs[1 - rd][g], c, st["l"],
                              plan_first if st["b"] is None else plan_loop, g, st["q"])
            if c == 2:
                nxt = st["a"] + G
                nxt = min(nxt, H - 1) if isinstance(nxt, int) else jnp.minimum(nxt, H - 1)
                stage_q(1 - rd, g, nxt, col)
            if c == NC - 1:
                l_scs[1 - rd][g][...] = jnp.concatenate(st["l"], axis=1)

        def step_b(st, c):
            g, rd = st["g"], st["rd"]
            pb = pltpu.bitcast(p_scs[rd][g][c * 64:(c + 1) * 64, :], bf16)
            vT = pltpu.bitcast(vT_sc[:, c * CK:(c + 1) * CK], bf16)
            oc = jnp.dot(vT, pb, preferred_element_type=f32)
            st["o"] = oc if st["o"] is None else oc + st["o"]
            if c == NC - 1:
                store_o(st["b"], st["o"], l_scs[rd][g][...])

        def run(streams):
            for st in streams:
                for c in range(NC):
                    step_a(st, c)
                    if st["b"] is not None:
                        step_b(st, c)

        def pre_emitter(heads, wsum, q_ref, restage):
            todo = [(h, t, (e + t) % E, e) for h in heads for e0 in range(0, E, 2) for t in range(NCOL)
                    for e in range(e0, min(e0 + 2, E))]
            cache = {}
            total = len(todo)
            quota = [0.0]
            lsum = {}

            def emit(w, lo=0, nslot=32):
                quota[0] += total * w / wsum
                n = min(int(quota[0] + 1e-6), len(todo), nslot - lo)
                quota[0] -= n
                outs = {}
                for k in range(n):
                    h, t, e, cnt = todo.pop(0)
                    if cnt % 2 == 0:
                        cache.clear()
                    p = jnp.exp2(vpu_scores(q_rows(cache, q_ref, h * DH, t), e))
                    pe_sc[h, e * 8:(e + 1) * 8, lanes(t)] = pack(p)
                    lv = jnp.sum(p.reshape(2, 8, 128), axis=0)
                    lsum[(h, t)] = lv if cnt == 0 else lsum[(h, t)] + lv
                    if cnt == E - 1:
                        le_sc[h, :, lanes(t)] = lsum[(h, t)]
                        if restage and t == NCOL - 1:
                            q_ref[h * DH:(h + 1) * DH, :] = load_qT(h, coln2).astype(f32)
                    outs[lo + ((2 * k + 1) * (nslot - lo)) // (2 * n)] = lv
                return outs
            return emit, todo

        def set_flag(t, qn):
            qmax = jnp.max(jnp.sum(qn, axis=0, keepdims=True)) * 1.02
            ok = qmax * kn_sc[0] <= S_BOUND * S_BOUND
            flag_sc[t] = ok.astype(jnp.int32)

        @pl.when(i == 0)
        def _():
            wk_copy.start()
            wv_copy.start()
            wq_copy.start()
            for t in range(NQ):
                x_copy(t).start()
            acc = {}
            emit0, todo0 = pre_emitter(range(NPV), (NQ - 1) * NCOL, qzero_sc, False)

            def proj(t):
                xt = x_sc[t * TQ:(t + 1) * TQ, :]
                if t == 0:
                    r = lax.dot_general(wT_sc[...], xt, NT, preferred_element_type=f32)
                else:
                    w_u32 = pltpu.bitcast(wT_sc[...], u32)
                    parts = []
                    for cc in range(NCOL):
                        outs = emit0(1, 8 if (t == 1 and cc == 0) else 0, NRW)
                        parts.append(lax.dot_general(anchored_lhs(w_u32, outs, i > 0), xt[lanes(cc), :], NT,
                                                     preferred_element_type=f32))
                    r = jnp.concatenate(parts, axis=1)
                kT = (r[0:DH, :] * scale).astype(bf16).astype(f32)
                k = kT.T
                k_sc[t * TQ // 2:(t + 1) * TQ // 2, :] = pltpu.bitcast(k.astype(bf16), u32)
                vb = r[DH:2 * DH, :].astype(bf16)
                vT_sc[:, t * TQ:(t + 1) * TQ] = pltpu.bitcast(vb, u32)
                kk2 = jnp.sum(kT * kT, axis=0, keepdims=True)
                va = jnp.abs(vb.astype(f32))
                acc["k"] = kk2 if t == 0 else jnp.maximum(acc["k"], kk2)
                acc["v"] = va if t == 0 else jnp.maximum(acc["v"], va)
                if t == 0:
                    for d in range(DH):
                        kb_sc[d] = jnp.broadcast_to(k[0:16 * NKB, d:d + 1], (16 * NKB, 128)).reshape(2 * NKB, 8, 128)
                qT = r[2 * DH:, :]
                for tt in range(NCOL):
                    qb = qT[:, lanes(tt)].astype(bf16)
                    cs = slice(t * TQ + tt * 128, t * TQ + (tt + 1) * 128)
                    qT_sc[:, cs] = pltpu.bitcast(qb, u32)
                    if t == 0:
                        qzero_sc[:, lanes(tt)] = qb[0:NPV * DH, :].astype(f32)
                    if t == 1:
                        qnext_sc[:, lanes(tt)] = qb.astype(f32)
                q4 = qT.reshape(H, 2, 8, TQ)
                qn_sc[t] = jnp.max(jnp.sum(q4 * q4, axis=1), axis=0)

            def pre_mxu(heads):
                kk = pltpu.bitcast(k_sc[0:8 * E, :], bf16)
                for h in heads:
                    p = jnp.exp2(jnp.dot(kk, load_qT(h, 0), preferred_element_type=f32))
                    for t in range(NCOL):
                        pe_sc[h, :, lanes(t)] = pack(p[:, lanes(t)])
                    le_sc[h] = jnp.sum(p.reshape(2 * E, 8, TQ), axis=0)

            wk_copy.wait()
            wv_copy.wait()
            wq_copy.wait()
            wT_sc[2 * DH:, :] = wq_sc[...].T
            x_copy(0).wait()
            proj(0)
            for t in range(1, NQ):
                x_copy(t).wait()
            for cp in late_copies:
                cp.start()
            for g in range(G):
                stage_q(1, g, g, 0)
            hs = list(range(NPV, H))
            n1 = min(4, len(hs))
            cuts = [n1 + ((len(hs) - n1) * t) // (NQ - 2) for t in range(NQ - 1)]
            pre_mxu(hs[:n1])
            for t in range(1, NQ):
                proj(t)
                if t < NQ - 1:
                    pre_mxu(hs[cuts[t - 1]:cuts[t]])
            assert not todo0
            kn_sc[0] = jnp.where(jnp.max(acc["v"]) <= V_BOUND, jnp.max(acc["k"]), jnp.inf)
            set_flag(0, qn_sc[0])

        fast = flag_sc[i] == 1

        @pl.when(fast)
        def _():
            run([stream(g, 1, g, None) for g in range(G)])

            def body(j, carry):
                for par in range(2):
                    @pl.when((j & 1) == par)
                    def _():
                        run([stream(g, par, (j + 1) * G + g, j * G + g) for g in range(G)])
                return carry
            lax.fori_loop(0, NIT, body, 0)

        @pl.when(jnp.logical_not(fast))
        def _():
            def gbody(head, carry):
                qT = load_qT(head, col)
                g = head % G

                def s_pass(c, mn):
                    kk = pltpu.bitcast(k_sc[pl.ds(pl.multiple_of(c * 64, 64), 64), :], bf16)
                    s = jnp.dot(kk, qT, preferred_element_type=f32)
                    s_sc[pl.ds(pl.multiple_of(c * CK, CK), CK), :] = s
                    return jnp.maximum(mn, jnp.max(s.reshape(CK // 8, 8, TQ), axis=0))
                mn = lax.fori_loop(0, NC, s_pass, jnp.full((8, TQ), -jnp.inf, f32))
                m = jnp.max(mn, axis=0, keepdims=True)

                def p_pass(c, carry2):
                    l, o = carry2
                    p = jnp.exp2(s_sc[pl.ds(pl.multiple_of(c * CK, CK), CK), :] - m)
                    l = l + jnp.sum(p.reshape(CK // 8, 8, TQ), axis=0)
                    pb = p.astype(bf16)
                    p_all[FPAR][g, pl.ds(pl.multiple_of(c * 64, 64), 64), :] = pltpu.bitcast(pb, u32)
                    vT = pltpu.bitcast(vT_sc[:, pl.ds(pl.multiple_of(c * CK, CK), CK)], bf16)
                    return l, o + jnp.dot(vT, pb, preferred_element_type=f32)
                l, o = lax.fori_loop(0, NC, p_pass,
                                     (jnp.zeros((8, TQ), f32), jnp.zeros((DH, TQ), f32)))
                l_all[FPAR][g] = l
                store_o(head, o, l)
                return carry
            lax.fori_loop(0, H, gbody, 0)

        @pl.when(i == 0)
        def _():
            for cp in late_copies:
                cp.wait()

        last = [stream(g, FPAR, None, H - G + g) for g in range(G)]
        pending = [(st, c) for st in last for c in range(NC)]

        def emit_b(n):
            for _ in range(min(n, len(pending))):
                step_b(*pending.pop(0))

        set_flag(inext, qn_sc[inext])
        for g in range(G):
            stage_q(1, g, g, coln)

        wts = [list(TIE) for _ in range(NF)]
        wts[0][0] *= 0.5
        for f in range(NF - GRP[-1], NF):
            wts[f][2] = 0
        emit_pre, todo = pre_emitter(range(H), sum(sum(w) for w in wts), qnext_sc, True)
        never = flag_sc[i] > 1

        xt = x_sc[pl.ds(col, TQ), :]
        x_u32 = pltpu.bitcast(xt, u32)
        gw = gw_sc[...].reshape(1, D).astype(f32)
        z = jnp.sum(xt.astype(f32) * gw, axis=-1, keepdims=True)
        gate = jnp.broadcast_to(jax.nn.sigmoid(z), (TQ, 128))
        a = None
        b = None
        f0 = 0
        for gidx, gn in enumerate(GRP):
            if gidx == WO_POS:
                emit_b(len(pending))
                a = lax.dot_general(oT_sc[...], wo_sc[...], TN, preferred_element_type=f32)
            hms = []
            for f in range(f0, f0 + gn):
                fs = slice(f * FC, (f + 1) * FC)
                lhs = anchored_lhs(x_u32, emit_pre(wts[f][0], 16 if f == 0 else 0), never)
                hg = 0.5 * jnp.dot(lhs, wg_sc[:, fs], preferred_element_type=f32)
                emit_b(NB)
                lhs = anchored_lhs(x_u32, emit_pre(wts[f][1]), never)
                u = jnp.dot(lhs, wu_sc[:, fs], preferred_element_type=f32)
                emit_b(NB)
                hms.append((hg + hg * jnp.tanh(hg)) * u)
            hm = jnp.concatenate(hms, axis=1).astype(bf16)
            nw = D // gn
            parts = []
            for k in range(gn):
                bc = jnp.dot(hm, wd_sc[f0 * FC:(f0 + gn) * FC, k * nw:(k + 1) * nw],
                             preferred_element_type=f32)
                outs = emit_pre(wts[f0 + k][2])
                if outs:
                    outs = {2 * r: v for r, v in outs.items()}
                    first = anchored(bc[:, 0:128], outs, never)
                    bc = first if nw == 128 else jnp.concatenate([first, bc[:, 128:]], axis=1)
                emit_b(NB)
                parts.append(bc)
            bc = jnp.concatenate(parts, axis=1)
            b = bc if b is None else b + bc
            f0 += gn
        assert a is not None and not todo and not pending
        g4 = jnp.concatenate([gate] * (D // 128), axis=1)
        o_ref[...] = (g4 * a + (1.0 - g4) * b).astype(o_ref.dtype)

    scratch = [
        pltpu.VMEM((D,), bf16),
        pltpu.VMEM((S, D), bf16),
        pltpu.VMEM((D, D), bf16),
        pltpu.VMEM((2 * DH + D, D), bf16),
        pltpu.VMEM((D, D), bf16),
        pltpu.VMEM((D, F), bf16),
        pltpu.VMEM((D, F), bf16),
        pltpu.VMEM((F, D), bf16),
        pltpu.VMEM((S // 2, DH), u32),
        pltpu.VMEM((DH // 2, S), u32),
        pltpu.VMEM((D // 2, S), u32),
        pltpu.VMEM((D, TQ), bf16),
        pltpu.VMEM((DH, NKB * 2, 8, 128), f32),
        pltpu.VMEM((S, TQ), f32),
        pltpu.VMEM((NQ, 8, TQ), f32),
        pltpu.VMEM((D, TQ), f32),
        pltpu.VMEM((NPV * DH, TQ), f32),
        pltpu.VMEM((H, 8 * E, TQ), u32),
        pltpu.VMEM((H, 8, TQ), f32),
        pltpu.SMEM((NQ,), jnp.int32),
        pltpu.SMEM((1,), f32),
        pltpu.SemaphoreType.DMA((NQ + 8,)),
    ]
    scratch += [pltpu.VMEM((G, S // 2, TQ), u32)] * 2 + [pltpu.VMEM((G, 8, TQ), f32)] * 2
    scratch += [pltpu.VMEM((DH, TQ), f32)] * (2 * G) + [pltpu.VMEM((DH // 2, TQ), u32)] * (2 * G)
    return kernel, scratch


_CFG = dict(TQ=512, FC=128, G=4, NB=2, WO_POS=3, NVG=19, NVGA=17, P0=-14, P1=8, E=5, TIE=(7, 6, 7), NPV=12, GRP=(4, 4, 4, 2))


@jax.jit
def pallas_gated_mix__grouped_kv_mqa__swiglu_ffn__prompt_kernel(
    A_x: jax.Array,
    A_wq: jax.Array,
    A_wk: jax.Array,
    A_wv: jax.Array,
    A_wo: jax.Array,
    B_x: jax.Array,
    B_w_gate: jax.Array,
    B_w_up: jax.Array,
    B_w_down: jax.Array,
    gate_w: jax.Array,
):
    del B_x
    B, S, D = A_x.shape
    F = B_w_gate.shape[1]
    TQ = _CFG["TQ"]
    kernel, scratch = _make_kernel(S, D, F, **_CFG)
    out = pl.pallas_call(
        kernel,
        grid=(S // TQ,),
        in_specs=[pl.BlockSpec(memory_space=pl.ANY)] * 9,
        out_specs=pl.BlockSpec((TQ, D), lambda i: (i, 0)),
        out_shape=jax.ShapeDtypeStruct((S, D), A_x.dtype),
        scratch_shapes=scratch,
        compiler_params=pltpu.CompilerParams(
            dimension_semantics=("arbitrary",),
            vmem_limit_bytes=100 * 1024 * 1024),
    )(A_x.reshape(S, D), A_wq, A_wk.T, A_wv.T, A_wo, B_w_gate, B_w_up, B_w_down, gate_w)
    return out.reshape(B, S, D)
```
